```python
import os as _os
_os.environ.setdefault("JAX_PLATFORMS", "cpu")
import jax
import jax.numpy as jnp

def _softmax(x, axis=-1):
    return jax.nn.softmax(x, axis=axis)
def _gelu(x):
    return jax.nn.gelu(x, approximate=True)
def _silu(x):
    return jax.nn.silu(x)
def _sigmoid(x):
    return jax.nn.sigmoid(x)
def _layernorm(x, axis=-1, eps=1e-5):
    m = jnp.mean(x, axis=axis, keepdims=True)
    v = jnp.var(x, axis=axis, keepdims=True)
    return (x - m) / jnp.sqrt(v + eps)
def _scatter_add(tgt, idx, src, axis=0):
    return tgt.at[idx].add(src)
def _segment_sum(src, seg, n):
    return jax.ops.segment_sum(src, seg, n)
class _Rng:
    def __init__(self, key):
        self._k = key
    def _next(self):
        self._k, sub = jax.random.split(self._k)
        return sub
    def normal(self, shape):
        return jax.random.normal(self._next(), shape, dtype=jnp.bfloat16)
    def randint(self, lo, hi, shape):
        return jax.random.randint(self._next(), shape, lo, hi, dtype=jnp.int32)
    def uniform(self, shape, lo=0.0, hi=1.0):
        return jax.random.uniform(self._next(), shape, jnp.bfloat16, lo, hi)
    def permutation(self, n):
        return jax.random.permutation(self._next(), n)


kernel_name = 'concat_heads__sliding_block__ssm_conv_s4__prompt'

def setup_inputs():
    _rng = _Rng(jax.random.key(int.from_bytes(__import__("os").urandom(4), "little")))
    _w = (lambda a: (lambda t: t.astype(jnp.bfloat16) if jnp.issubdtype(t.dtype, jnp.floating) else t)(jnp.asarray(a)))
    def _A_setup():
        B, S, D = 1, 2048, 512
        return {
            "x": _w((lambda *s: _rng.normal(s) * 0.2)(B, S, D)),
            "wqkv": _w((lambda *s: _rng.normal(s) * 0.2)(D, 3 * D)),
            "wo": _w((lambda *s: _rng.normal(s) * 0.05)(D, D)),
        }
    _A_in = _A_setup()

    def _B_setup():
        B, L, D, N = 1, 2048, 512, 128
        A_re = -jnp.exp((lambda *s: _rng.normal(s) * 0.8)(D, N))
        A_im = jnp.pi * (lambda *s: _rng.normal(s) * 0.8)(D, N)
        B_re = (lambda *s: _rng.normal(s) * 0.8)(D, N)
        B_im = (lambda *s: _rng.normal(s) * 0.8)(D, N)
        C_re = (lambda *s: _rng.normal(s) * 0.8)(D, N)
        C_im = (lambda *s: _rng.normal(s) * 0.8)(D, N)
        log_dt = (lambda *s: _rng.normal(s) * 0.8)(D) * 0.5 - 4.0
        Dskip = (lambda *s: _rng.normal(s) * 0.05)(D)
        return {
            "u": _w((lambda *s: _rng.normal(s) * 0.05)(B, L, D)),
            "A_re": _w(A_re),
            "A_im": _w(A_im),
            "B_re": _w(B_re),
            "B_im": _w(B_im),
            "C_re": _w(C_re),
            "C_im": _w(C_im),
            "log_dt": _w(log_dt),
            "Dskip": _w(Dskip),
        }
    _B_in = _B_setup()

    return {
        "A_x": _A_in["x"],
        "A_wqkv": _A_in["wqkv"],
        "A_wo": _A_in["wo"],
        "B_u": _B_in["u"],
        "B_A_re": _B_in["A_re"],
        "B_A_im": _B_in["A_im"],
        "B_B_re": _B_in["B_re"],
        "B_B_im": _B_in["B_im"],
        "B_C_re": _B_in["C_re"],
        "B_C_im": _B_in["C_im"],
        "B_log_dt": _B_in["log_dt"],
        "B_Dskip": _B_in["Dskip"],
    }

def reference(A_x, A_wqkv, A_wo, B_u, B_A_re, B_A_im, B_B_re, B_B_im, B_C_re, B_C_im, B_log_dt, B_Dskip):
    def _A_ref(x, wqkv, wo):
        B, S, D = x.shape
        H = 32; Dh = D // H; W = 256
        qkv = (lambda x, *d: x.transpose(*d))((x @ wqkv).reshape(B, S, 3, H, Dh), 2, 0, 3, 1, 4)
        q, k, v = qkv[0], qkv[1], qkv[2]
        scores = jnp.einsum("bhqd,bhkd->bhqk", q, k) * (Dh ** -0.5)
        idx = jnp.arange(S)
        mask = (idx[:, None] - idx[None, :] >= 0) & (idx[:, None] - idx[None, :] < W)
        scores = jnp.where(mask[None, None], scores, -1e9)
        p = _softmax(scores, axis=-1)
        o = jnp.einsum("bhqk,bhkd->bhqd", p, v)
        return (lambda x, *d: x.transpose(*d))(o, 0, 2, 1, 3).reshape(B, S, D) @ wo

    def _B_ref(u, A_re, A_im, B_re, B_im, C_re, C_im, log_dt, Dskip):
        Bsz, L, D = u.shape
        dt = jnp.exp(log_dt)[:, None]
        A = A_re + 1j * A_im
        Bc = B_re + 1j * B_im
        Cc = C_re + 1j * C_im
        logdA = dt * A
        dB = dt * Bc
        l = (lambda x, dt: x.astype(dt))(jnp.arange(L), A_re.dtype)
        P = jnp.exp(logdA[:, :, None] * l[None, None, :])
        K = jnp.einsum("dn,dnl,dn->dl", Cc, P, dB).real
        L2 = 2 * L
        Kp = jnp.pad(K, ((0, 0), (0, L)))
        up = (lambda x, *d: x.transpose(*d))(u, 0, 2, 1)
        up = jnp.pad(up, ((0, 0), (0, 0), (0, L)))
        Kf = (lambda x, axes=(-2,-1): jnp.fft.rfft2(x.astype(jnp.float32), axes=axes))(Kp[:, None, :], axes=(-2, -1))
        Uf = (lambda x, axes=(-2,-1): jnp.fft.rfft2(x.astype(jnp.float32), axes=axes))(up[:, :, None, :], axes=(-2, -1))
        Yf = Uf * Kf[None, :, :, :]
        y = (lambda x, s, axes=(-2,-1): jnp.fft.irfft2(x, s=s, axes=axes).astype(jnp.bfloat16))(Yf, (1, L2), axes=(-2, -1))[:, :, 0, :L]
        y = (lambda x, *d: x.transpose(*d))(y, 0, 2, 1) + u * Dskip[None, None, :]
        return y

    a = _A_ref(A_x, A_wqkv, A_wo)
    b = _B_ref(B_u, B_A_re, B_A_im, B_B_re, B_B_im, B_C_re, B_C_im, B_log_dt, B_Dskip)
    return jnp.concatenate([a, b], axis=-1)
```

```python
import functools
import numpy as np
import jax
import jax.numpy as jnp
from jax import lax
from jax.experimental import pallas as pl
from jax.experimental.pallas import tpu as pltpu

f32 = jnp.float32
bf16 = jnp.bfloat16
i32 = jnp.int32

S_LEN, D_MOD, N_ST = 2048, 512, 128
PITCH = 257
G = 4
NSS = 8
SCALE = float(0.25 * np.log2(np.e))
NEG = -1e30
RINGS = (3, 6, 2, 2, 3, 2, 2)
UB = 6


def cmul(ar, ai, br, bi):
    return ar * br - ai * bi, ar * bi + ai * br


def csq(ar, ai):
    return ar * ar - ai * ai, (ar + ar) * ai


def bc16(x):
    return pltpu.bitcast(x, bf16)


def toi(x):
    return pltpu.bitcast(x, i32)


def pk(a, b):
    return pltpu.bitcast(pltpu.pack_elementwise([a, b], packed_dtype=bf16), i32)


def srl(x, n):
    return lax.shift_right_logical(x, jnp.int32(n))


def rowb(ref, base, r):
    return jnp.take_along_axis(ref[pl.ds(base, 8), :], jnp.full((8, 128), r, i32), axis=0)


def slot_of_chunk(m):
    p, m2 = m % 2, m // 2
    return 16 * p + 2 * (m2 % 8) + m2 // 8


def ssm_prep(p, dt, dsc):
    lr = dt * p["Ar"]
    li = dt * p["Ai"]
    cr, ci = cmul(p["Cr"], p["Ci"], dt * p["Br"], dt * p["Bi"])
    eh = jnp.exp(lr * 0.5)
    th = li * 0.5
    whr = eh * jnp.cos(th)
    whi = eh * jnp.sin(th)
    mx = jnp.maximum(jnp.abs(cr), jnp.abs(ci))
    pos = mx > 0
    mxs = jnp.where(pos, mx, 1.0)
    inv = 1.0 / mxs
    a = cr * inv
    b = ci * inv
    h = jnp.sqrt(a * a + b * b)
    t = jnp.sqrt(jnp.where(pos, (h + jnp.abs(a)) * 0.5, 1.0))
    q = b * (0.5 / t)
    sm = jnp.where(pos, jnp.sqrt(mxs), 0.0)
    sr = jnp.where(a >= 0, t, jnp.abs(q)) * sm
    si = jnp.where(a >= 0, q, jnp.where(b < 0, -t, t)) * sm
    g0 = cmul(sr, si, whr, whi)
    w1 = csq(whr, whi)
    w2 = csq(*w1)
    w4 = csq(*w2)
    w8 = csq(*w4)
    w16 = csq(*w8)
    w32 = csq(*w16)
    w64 = csq(*w32)
    B = [None] * 8
    B[0] = g0
    B[1] = cmul(*B[0], *w2)
    B[2] = cmul(*B[0], *w4)
    B[3] = cmul(*B[1], *w4)
    for k in range(4):
        B[4 + k] = cmul(*B[k], *w8)
    k0 = jnp.sum(cr, axis=1, keepdims=True) + dsc
    dg = jnp.broadcast_to(k0, cr.shape)
    return B, w1, w16, w64, pk(dg, dg)


def kernel(x_hbm, w_hbm, wo_hbm, u_hbm, Ar_h, Ai_h, Br_h, Bi_h, Cr_h, Ci_h, ldt_h, dsk_h, o_hbm,
           zs, x_v, w_v, wo_v, u_v, par_v, ldt_v, dsk_v, oa_v, ob_v,
           wqvT, wk_i, wo_i, K_s, VT_s, QT_s, OT_s, mk_s,
           bbr, bbi, w1r, w1i, w16r, w16i, w64r, w64i, dgs, ut, yt, colt,
           sem_in, sem_par, sem_oa, sem_ob, *scr):
    it_ = iter(scr)
    s_refs = [next(it_) for _ in range(NSS)]
    RT, RL, RS, RZ, RY, RK, RTT = [[next(it_) for _ in range(n)] for n in RINGS]

    par_h = (Ar_h, Ai_h, Br_h, Bi_h, Cr_h, Ci_h)
    cp_small = [pltpu.make_async_copy(ldt_h, ldt_v, sem_par.at[0]),
                pltpu.make_async_copy(dsk_h, dsk_v, sem_par.at[1])]
    cp_par = [pltpu.make_async_copy(par_h[k], par_v.at[k], sem_par.at[2 + k]) for k in range(6)]
    cp_u = pltpu.make_async_copy(u_hbm, u_v, sem_in.at[0])
    cp_w = pltpu.make_async_copy(w_hbm, w_v, sem_in.at[1])
    cp_x = pltpu.make_async_copy(x_hbm, x_v, sem_in.at[2])
    cp_wo = pltpu.make_async_copy(wo_hbm, wo_v, sem_in.at[3])
    for c in cp_small + cp_par + [cp_u, cp_w, cp_x, cp_wo]:
        c.start()

    def zinit(i, c):
        zs[i] = 0
        return c
    lax.fori_loop(0, 2, zinit, 0)
    z0 = pl.multiple_of(zs[0], 128)
    z1 = pl.multiple_of(zs[1], 128)

    lane = lax.broadcasted_iota(i32, (8, 128), 1)
    sub = lax.broadcasted_iota(i32, (8, 128), 0)
    rev = 7 - sub

    for c in cp_small:
        c.wait()
    dtrow = jnp.exp(ldt_v[...].reshape(1, 512).astype(f32)).astype(bf16).astype(f32)
    dsrow = dsk_v[...].reshape(1, 512).astype(f32)
    for k in range(4):
        colt[128 * k:128 * (k + 1), 0:128] = jnp.broadcast_to(dtrow[:, 128 * k:128 * (k + 1)], (128, 128)).T
        colt[128 * k:128 * (k + 1), 128:256] = jnp.broadcast_to(dsrow[:, 128 * k:128 * (k + 1)], (128, 128)).T
    for c in cp_par:
        c.wait()
    RB = 64

    def prep_body(it, c):
        r0 = pl.multiple_of(it * RB, RB)
        names = ("Ar", "Ai", "Br", "Bi", "Cr", "Ci")
        p = {n: par_v[k, pl.ds(r0, RB), :].astype(f32) for k, n in enumerate(names)}
        B, w1, w16, w64, dg = ssm_prep(p, colt[pl.ds(r0, RB), 0:128], colt[pl.ds(r0, RB), 128:129])
        for s in range(8):
            for gg in range(RB // 8):
                bbr[pl.ds(9 * (r0 + 8 * gg) + s, 8, stride=9), :] = B[s][0][8 * gg:8 * gg + 8]
                bbi[pl.ds(9 * (r0 + 8 * gg) + s, 8, stride=9), :] = B[s][1][8 * gg:8 * gg + 8]
        w1r[pl.ds(r0, RB), :] = w1[0]
        w1i[pl.ds(r0, RB), :] = w1[1]
        w16r[pl.ds(r0, RB), :] = w16[0]
        w16i[pl.ds(r0, RB), :] = w16[1]
        w64r[pl.ds(r0, RB), :] = w64[0]
        w64i[pl.ds(r0, RB), :] = w64[1]
        dgs[pl.ds(r0, RB), :] = dg
        return c
    lax.fori_loop(0, 512 // RB, prep_body, 0)

    cp_u.wait()

    def ut_body(m2, c):
        for db in range(4):
            xi = toi(u_v[pl.ds(pl.multiple_of(m2 * 128, 128), 128), 128 * db:128 * (db + 1)])
            pcs = []
            for v2 in range(8):
                v = (v2 // 4) * 4 + (3 - v2 % 4)
                t = jnp.take_along_axis(xi[8 * v:8 * v + 8], rev, axis=0)
                pcs.append((t << 16) | srl(t, 16))
            x = bc16(jnp.concatenate(pcs, axis=0))
            ut[pl.ds(m2 * PITCH + 64 * db, 64), :] = toi(x.T)
        return c
    lax.fori_loop(0, 16, ut_body, 0)

    def stageA(g, ts, ls, ss):
        gb = pl.multiple_of(g * 8, 8)
        for r in range(8):
            e0 = (bbr[pl.ds(9 * gb + 9 * r, 8), :], bbi[pl.ds(9 * gb + 9 * r, 8), :])
            w1 = (rowb(w1r, gb, r), rowb(w1i, gb, r))
            w16 = (rowb(w16r, gb, r), rowb(w16i, gb, r))
            e1 = cmul(*e0, *w1)
            vr = []
            vi = []
            for a in range(4):
                vr.append(pk(e0[0], e1[0]))
                vi.append(pk(e0[1], e1[1]))
                if a < 3:
                    e0 = cmul(*e0, *w16)
                    e1 = cmul(*e1, *w16)
            Vr = jnp.concatenate(vr, 0)
            Vi = jnp.concatenate(vi, 0)
            ts[pl.ds(z0 + 64 * r, 32), :] = Vr
            ts[pl.ds(z0 + 64 * r + 32, 32), :] = Vi
            if r % 2 == 0:
                dp = g * 4 + r // 2
                A_ = ut[pl.ds(dp, 8, stride=PITCH), :]
                B_ = ut[pl.ds(dp + 8 * PITCH, 8, stride=PITCH), :]
                X = (A_ & 0xFFFF) | (B_ << 16)
            else:
                X = srl(A_, 16) | (B_ & jnp.int32(-65536))
            L = jnp.concatenate([jnp.where(lane < 64, X, 0), jnp.where(lane >= 64, X, 0)], 0)
            ls[pl.ds(z0 + 16 * r, 16), :] = L
            Lb = bc16(L)
            Sr = jnp.dot(Lb, bc16(jnp.concatenate([Vr, Vr], 0)), preferred_element_type=f32)
            Si = jnp.dot(Lb, bc16(jnp.concatenate([Vi, Vi], 0)), preferred_element_type=f32)
            ss[pl.ds(z0 + 66 * r, 32), :] = Sr
            ss[pl.ds(z0 + 66 * r + 33, 32), :] = Si

    def stageB(g, ss, zz):
        gb = pl.multiple_of(g * 8, 8)
        wr = w64r[pl.ds(gb, 8), :]
        wi = w64i[pl.ds(gb, 8), :]
        zr = zi = None
        for m in range(32):
            s = slot_of_chunk(m)
            if m == 0:
                zz[pl.ds(z0 + s, 8, stride=66), :] = bbr[pl.ds(9 * gb, 8, stride=9), :]
                zz[pl.ds(z0 + 33 + s, 8, stride=66), :] = bbi[pl.ds(9 * gb, 8, stride=9), :]
            else:
                zz[pl.ds(z0 + s, 8, stride=66), :] = zr
                zz[pl.ds(z0 + 33 + s, 8, stride=66), :] = zi
            if m < 31:
                sr = ss[pl.ds(z1 + s, 8, stride=66), :]
                si = ss[pl.ds(z1 + 33 + s, 8, stride=66), :]
                if m == 0:
                    zr, zi = sr, si
                else:
                    tr, ti = cmul(zr, zi, wr, wi)
                    zr = tr + sr
                    zi = ti + si

    mdiag = [jnp.where(lane == 63 - 16 * a - 2 * sub, jnp.int32(0xFFFF), 0)
             | jnp.where(lane == 62 - 16 * a - 2 * sub, jnp.int32(-65536), 0) for a in range(4)]

    def stageC1(g, ts, zz, ys, ks):
        nt = (((1,), (1,)), ((), ()))
        for r in range(8):
            Vr = bc16(ts[pl.ds(z1 + 64 * r, 32), :])
            Vi = bc16(ts[pl.ds(z1 + 64 * r + 32, 32), :])
            Zr = zz[pl.ds(z1 + 66 * r, 32), :].astype(bf16)
            Zi = zz[pl.ds(z1 + 66 * r + 33, 32), :].astype(bf16)
            yi = (lax.dot_general(Zr, Vr, nt, preferred_element_type=f32)
                  - lax.dot_general(Zi, Vi, nt, preferred_element_type=f32))
            ks[pl.ds(z0 + 8 * r, 8), :] = jnp.concatenate([yi[0:8], jnp.zeros((8, 64), f32)], axis=1)
            y0 = jnp.where(sub[:, :64] == 0, 0.0, yi[0:8])
            ys[pl.ds(z0 + 32 * r, 32), 0:64] = jnp.concatenate([y0, yi[8:32]], 0)

    def stageC2(g, ks, tts):
        gb = pl.multiple_of(g * 8, 8)
        for r in range(8):
            k1 = jnp.take_along_axis(ks[pl.ds(z1 + 8 * r, 8), :], jnp.zeros((8, 128), i32), axis=0)
            src = pk(pltpu.roll(k1, 1, 1), k1)
            dg = rowb(dgs, gb, r)
            T = []
            for a in range(4):
                t = pltpu.roll(src, 49 - 16 * a, 1, stride=2, stride_axis=0)
                t = jnp.take_along_axis(t, rev, axis=0)
                T.append(t | (dg & mdiag[a]))
            tts[pl.ds(z0 + 32 * r, 32), :] = jnp.concatenate(T, 0)

    def stageC3(g, ls, tts, ys):
        for r in range(8):
            T = tts[pl.ds(z1 + 32 * r, 32), :]
            Lb = bc16(ls[pl.ds(z1 + 16 * r, 16), :])
            yt_ = jnp.dot(Lb, bc16(jnp.concatenate([T, T], 0))[:, :64], preferred_element_type=f32)
            y = ys[pl.ds(z1 + 32 * r, 32), 0:64] + yt_
            yf = jnp.concatenate([y[0:16], y[16:32]], axis=1)
            if r % 2 == 0:
                ye = yf
            else:
                w = pk(ye, yf)
                dp = g * 4 + r // 2
                yt[pl.ds(dp, 8, stride=PITCH), :] = w[0:8]
                yt[pl.ds(dp + 8 * PITCH, 8, stride=PITCH), :] = w[8:16]

    NG = 64
    ORDER = ("C3", "A", "C1", "C2", "B")

    def step(t, tm, lo, hi):
        def ok(k):
            return (lo is None or tm - k >= lo) and (hi is None or tm - k < hi)
        for st in ORDER:
            if st == "A" and ok(0):
                stageA(t, RT[tm % len(RT)], RL[tm % len(RL)], RS[tm % len(RS)])
            if st == "B" and ok(1):
                stageB(t - 1, RS[(tm - 1) % len(RS)], RZ[(tm - 1) % len(RZ)])
            if st == "C1" and ok(2):
                stageC1(t - 2, RT[(tm - 2) % len(RT)], RZ[(tm - 2) % len(RZ)], RY[(tm - 2) % len(RY)],
                        RK[(tm - 2) % len(RK)])
            if st == "C2" and ok(3):
                stageC2(t - 3, RK[(tm - 3) % len(RK)], RTT[(tm - 3) % len(RTT)])
            if st == "C3" and ok(4):
                stageC3(t - 4, RL[(tm - 4) % len(RL)], RTT[(tm - 4) % len(RTT)], RY[(tm - 4) % len(RY)])

    DEP = 4
    for t in range(DEP):
        step(t, t, 0, None)
    nloop = (NG - DEP) // UB

    def bbody(it, c):
        t = DEP + it * UB
        for j in range(UB):
            step(t + j, DEP + j, None, None)
        return c
    lax.fori_loop(0, nloop, bbody, 0)
    for t in range(DEP + nloop * UB, NG + DEP):
        step(t, t, None, NG)

    def fin_body(rho, c):
        m2 = rho // 2 + 8 * (rho % 2)
        for db in range(4):
            x = bc16(yt[pl.ds(rho * PITCH + 64 * db, 64), :])
            ob_v[pl.ds(pl.multiple_of(m2 * 128, 128), 128), 128 * db:128 * (db + 1)] = x.T
        return c
    lax.fori_loop(0, 16, fin_body, 0)
    cp_ob = pltpu.make_async_copy(ob_v, o_hbm.at[:, 512:1024], sem_ob.at[0])
    cp_ob.start()

    r_ = lax.broadcasted_iota(i32, (128, 128), 0)
    c_ = lax.broadcasted_iota(i32, (128, 128), 1)
    mk_s[...] = jnp.where(r_ <= c_, 1.0, 0.0).astype(f32)
    cp_w.wait()
    cp_wo.wait()
    for ct in range(4):
        for ht in range(8):
            col = ht * 128 if ht < 4 else 512 + ht * 128
            wqvT[ht * 64:(ht + 1) * 64, ct * 128:(ct + 1) * 128] = toi(w_v[ct * 128:(ct + 1) * 128, col:col + 128].T)
        wk_i[ct * 64:(ct + 1) * 64, :] = toi(w_v[ct * 128:(ct + 1) * 128, 512:1024])
        wo_i[ct * 64:(ct + 1) * 64, :] = toi(wo_v[ct * 128:(ct + 1) * 128, :])
    cp_x.wait()
    nt = (((1,), (1,)), ((), ()))

    def projK(i):
        xb = x_v[pl.ds(pl.multiple_of(i * 128, 128), 128), :]
        k = jnp.dot(xb, bc16(wk_i[...]), preferred_element_type=f32)
        K_s[pl.ds(pl.multiple_of(i * 64, 64), 64), :] = toi(k.astype(bf16))

    def projQV(i, ch):
        xb = x_v[pl.ds(pl.multiple_of(i * 128, 128), 128), :]
        w = bc16(wqvT[ch * 128:(ch + 1) * 128, :])
        t = lax.dot_general(w, xb, nt, preferred_element_type=f32)
        if ch < 2:
            QT_s[ch * 128:(ch + 1) * 128, pl.ds(pl.multiple_of(i * 128, 128), 128)] = toi((t * SCALE).astype(bf16))
        else:
            VT_s[(ch - 2) * 128:(ch - 1) * 128, pl.ds(pl.multiple_of(i * 128, 128), 128)] = toi(t.astype(bf16))

    def cp_oa(i):
        rows = pl.ds(pl.multiple_of(i * 128, 128), 128)
        return pltpu.make_async_copy(oa_v.at[rows, :], o_hbm.at[rows, 0:512], sem_oa.at[i])

    def outp(i):
        ot = bc16(OT_s[:, pl.ds(pl.multiple_of(i * 128, 128), 128)])
        o = lax.dot_general(ot, bc16(wo_i[...]), (((0,), (0,)), ((), ())), preferred_element_type=f32)
        oa_v[pl.ds(pl.multiple_of(i * 128, 128), 128), :] = o.astype(bf16)
        cp_oa(i).start()

    def attn(i, kind, extras):
        q0 = pl.multiple_of(i * 128, 128)
        kh = pl.multiple_of(i * 64 - 64 * kind, 64)
        ms = {}

        def stage1(h):
            s_s = s_refs[h % NSS]
            g, hh = h // 8, h % 8
            qh = bc16(QT_s[h * 8:(h + 1) * 8, pl.ds(q0, 128)])
            parts = []
            if hh > 0:
                parts.append(jnp.zeros((16 * hh, 128), bf16))
            parts.append(qh)
            if hh < 7:
                parts.append(jnp.zeros((16 * (7 - hh), 128), bf16))
            W = jnp.concatenate(parts, 0)
            gs = slice(g * 128, (g + 1) * 128)
            m = None
            if kind == 2:
                pcs = []
                for a in range(8):
                    pcs.append(K_s[pl.ds(kh + 8 * a, 8), gs])
                    pcs.append(K_s[pl.ds(kh + 128 + 8 * a, 8), gs])
                pcs.append(K_s[pl.ds(kh + 64, 64), gs])
                st = jnp.dot(bc16(jnp.concatenate(pcs, 0)), W, preferred_element_type=f32)
                for a in range(8):
                    t = jnp.where(mk_s[16 * a:16 * a + 16, :] > 0.5, st[32 * a + 16:32 * a + 32], st[32 * a:32 * a + 16])
                    s_s[pl.ds(z0 + 16 * a, 16), :] = t
                    mi = jnp.maximum(t[0:8], t[8:16])
                    m = mi if m is None else jnp.maximum(m, mi)
                mid = st[256:384]
            else:
                st = jnp.dot(bc16(K_s[pl.ds(kh, 64 * (kind + 1)), gs]), W, preferred_element_type=f32)
                dg = st[128 * kind:128 * kind + 128]
                for a in range(8):
                    t = jnp.where(mk_s[16 * a:16 * a + 16, :] > 0.5, dg[16 * a:16 * a + 16], NEG)
                    s_s[pl.ds(z0 + 16 * a, 16), :] = t
                    mi = jnp.maximum(t[0:8], t[8:16])
                    m = mi if m is None else jnp.maximum(m, mi)
                mid = st[0:128] if kind == 1 else None
            if mid is not None:
                s_s[pl.ds(z0 + 128, 128), :] = mid
                for a in range(16):
                    m = jnp.maximum(m, mid[8 * a:8 * a + 8])
            ms[h] = jnp.max(m, axis=0, keepdims=True)

        def stage2(h):
            s_s = s_refs[h % NSS]
            m = ms[h]
            a = jnp.exp2(s_s[pl.ds(z1, 128), :] - m)
            l = jnp.sum(a, axis=0, keepdims=True)
            if kind >= 1:
                b = jnp.exp2(s_s[pl.ds(z1 + 128, 128), :] - m)
                l = l + jnp.sum(b, axis=0, keepdims=True)
            if kind == 2:
                ad = a * mk_s[...]
                p = jnp.concatenate([a - ad, b, ad], 0)
            elif kind == 1:
                p = jnp.concatenate([b, a], 0)
            else:
                p = a
            vt = bc16(VT_s[h * 8:(h + 1) * 8, pl.ds(pl.multiple_of(i * 128 - 128 * kind, 128), 128 * (kind + 1))])
            ot = jnp.dot(vt, p.astype(bf16), preferred_element_type=f32) * (1.0 / l)
            OT_s[h * 8:(h + 1) * 8, pl.ds(q0, 128)] = toi(ot.astype(bf16))

        R = 32 // G
        ex = list(extras)
        for t in range(R + 1):
            if t < R:
                for j in range(G):
                    stage1(t * G + j)
            if t == R:
                while ex:
                    ex.pop(0)()
            if t >= 1:
                for j in range(G):
                    stage2((t - 1) * G + j)

    def P(i):
        return [lambda: projK(i)] + [functools.partial(projQV, i, ch) for ch in range(4)]

    def O(i):
        return [lambda: outp(i)]

    for f in P(0):
        f()
    attn(0, 0, P(1))
    attn(1, 1, P(2) + O(0))

    def abody(i, c):
        attn(i, 2, P(i + 1) + O(i - 1))
        return c
    lax.fori_loop(2, 15, abody, 0)
    attn(15, 2, O(14))
    outp(15)

    cp_ob.wait()

    def wbody(i, c):
        cp_oa(i).wait()
        return c
    lax.fori_loop(0, 16, wbody, 0)


@jax.jit
def pallas_concat_heads__sliding_block__ssm_conv_s4__prompt_kernel(
    A_x, A_wqkv, A_wo, B_u, B_A_re, B_A_im, B_B_re, B_B_im, B_C_re, B_C_im, B_log_dt, B_Dskip,
):
    V = pltpu.VMEM
    scr = [
        pltpu.SMEM((2,), i32),
        V((S_LEN, 512), bf16), V((512, 1536), bf16), V((512, 512), bf16), V((S_LEN, 512), bf16),
        V((6, 512, 128), bf16), V((512,), bf16), V((512,), bf16), V((S_LEN, 512), bf16), V((S_LEN, 512), bf16),
        V((512, 512), i32), V((256, 512), i32), V((256, 512), i32), V((1024, 512), i32),
        V((256, 2048), i32), V((256, 2048), i32), V((256, 2048), i32), V((128, 128), f32),
        V((512 * 9, 128), f32), V((512 * 9, 128), f32)] + [V((512, 128), f32)] * 6 + [
        V((512, 128), i32), V((16 * PITCH, 128), i32), V((16 * PITCH, 128), i32), V((512, 256), f32),
        pltpu.SemaphoreType.DMA((4,)), pltpu.SemaphoreType.DMA((8,)), pltpu.SemaphoreType.DMA((16,)),
        pltpu.SemaphoreType.DMA((1,)),
    ]
    scr += [V((256, 128), f32)] * NSS
    shp = [V((8 * 64, 128), i32), V((8 * 16, 128), i32), V((8 * 66, 128), f32), V((8 * 66, 128), f32),
           V((8 * 32, 128), f32), V((8 * 8, 128), f32), V((8 * 32, 128), i32)]
    for sh, n in zip(shp, RINGS):
        scr += [sh] * n
    out = pl.pallas_call(
        kernel,
        out_shape=jax.ShapeDtypeStruct((S_LEN, 1024), bf16),
        in_specs=[pl.BlockSpec(memory_space=pl.ANY)] * 12,
        out_specs=pl.BlockSpec(memory_space=pl.ANY),
        scratch_shapes=scr,
        compiler_params=pltpu.CompilerParams(vmem_limit_bytes=100 * 1024 * 1024),
        name="fused",
    )(A_x.reshape(S_LEN, 512), A_wqkv, A_wo, B_u.reshape(S_LEN, 512), B_A_re, B_A_im, B_B_re, B_B_im,
      B_C_re, B_C_im, B_log_dt, B_Dskip)
    return out.reshape(1, S_LEN, 1024)
```

```python
import functools
import numpy as np
import jax
import jax.numpy as jnp
from jax import lax
from jax.experimental import pallas as pl
from jax.experimental.pallas import tpu as pltpu

f32 = jnp.float32
bf16 = jnp.bfloat16
i32 = jnp.int32

S_LEN = 2048
PITCH = 261
NSS = 16
NA = 144
NGI = 5
SCALE = float(0.25 * np.log2(np.e))
NEG = -1e30
LOOK = 2
NACC = 2
SEQS = {
    'it0': (
        'WQ0 PW0 KA0 VA0 QA0 WQ1 WX S1_0 PW1 S1_1 S1_2 S1_3 S1_4 KA1 S1_5 VA1 QA1 K0 S1_6 S1_7 S2_0 Q0 S2_1 '
        'V1 S2_2 S2_3 V0 S1_8 S1_9 S1_11 S1_10 S2_4 S2_5 S2_6 S2_7 WQ2 WQ3 S1_13 S1_12 S1_14 PW2 PW3 S1_15 '
        'KA2 VA3 KA3 Q1 S2_8 S2_9 S2_10 S2_11 S2_12 S2_14 S2_13 S2_15 QA2 VA2 K1 S1_16 S1_17 S1_18 S1_19 K2 '
        'S1_20 QA3 S1_21 S1_22 S1_23 S2_16 S2_17 S2_18 K3 S2_19 V2 S1_25 S1_26 S1_27 S1_24 S2_20 S2_21 S2_22 '
        'S2_23 Q2 S1_28 S1_29 S1_30 S1_31 S2_24 S2_25 Q3 S2_27 S2_26 V3 S2_29 S2_30 S2_31 S2_28 ').split(),
    'it1': (
        'S1_3 S1_1 S1_0 S1_2 WA WOP COLT K0 S1_8 U0 S1_5 U1 PRE U2 U3 S1_4 S2_1 S1_7 K1 BA_0 BA_1 S2_0 S2_2 '
        'BA_2 S2_3 S1_6 S1_9 S1_11 BA_3 K2 S2_4 BB_0 S2_6 S2_7 S2_5 S1_10 S1_12 S1_15 S1_13 S1_14 BB_1 Q0 '
        'S2_8 S2_9 S2_10 K3 S2_11 S2_14 S1_17 S1_18 S1_16 S1_21 S1_19 BC1_2 BC1_3 BC2_3 S2_12 S2_13 BC1_1 '
        'S2_15 S1_20 BC1_0 S1_22 BC2_0 S2_17 S1_23 Q1 S2_16 O0 S2_19 S1_24 S1_25 S2_18 S1_27 S1_26 Q2 BC2_1 '
        'BC2_2 BC3_3 BC3_0 BC3_2 S2_20 BC3_1 S2_21 S2_22 S2_23 S1_28 S1_29 S1_30 S1_31 O1 S2_24 Q3 S2_25 PREP '
        'S2_26 S2_28 S2_27 S2_29 S2_30 S2_31 W1 ').split(),
    'it14': (
        'F0 K0 S1_2 S1_0 S1_1 S1_3 Q1 S2_2 F2 S1_4 S1_5 O0 S1_6 S1_7 K2 K3 S2_0 S2_3 S2_1 S1_8 S1_11 S1_9 '
        'S1_10 S2_4 S2_6 S2_7 S2_5 K1 Q3 S1_12 S1_13 S2_8 S1_14 S1_15 F1 S2_10 S1_16 S2_11 S1_17 S2_9 S1_19 '
        'S1_18 S2_12 S2_13 F3 O1 S1_20 S2_15 S2_14 S1_22 S1_23 S1_21 S2_16 S2_17 S2_18 S2_19 S1_26 S1_24 '
        'S1_25 S1_27 Q0 S2_20 S2_21 S2_22 S2_23 S1_28 S1_29 S1_30 S1_31 S2_25 S2_24 Q2 S2_27 S2_29 S2_26 '
        'S2_30 S2_31 S2_28 ').split(),
    'a': (
        'WU S1_2 K3 BA_1 S1_0 S1_3 S1_1 BA_2 S2_2 S1_7 S1_5 S1_4 S1_6 S2_3 S2_0 S2_1 BA_3 S1_8 BA_4 PR_4 BA_0 '
        'S1_9 PR_1 K0 S1_10 K2 S1_11 BB_0 PR_2 BB_1 Q0 PR_3 S2_4 K1 PR_0 BC1_3 BC1_2 BC1_4 S2_5 S2_6 S1_13 '
        'S1_12 S1_14 S2_7 S1_15 BC1_0 S2_10 U1 S2_11 U3 BC1_1 S2_8 U0 BC2_1 S2_9 S1_18 S1_17 U2 S1_16 S1_19 '
        'S2_15 BC2_4 BC2_3 S2_13 Q2 S2_12 S2_14 S1_20 BC2_0 S1_22 S2_17 S1_21 S1_23 S2_18 Q1 S2_19 S2_16 '
        'S1_27 S1_25 O0 S1_26 BC2_2 S2_22 S2_20 S1_24 BC3_4 S2_23 BC3_0 BC3_1 BC3_2 S1_28 S2_21 S1_31 S1_30 '
        'S1_29 BC3_3 O1 S2_24 S2_27 Q3 S2_26 S2_28 S2_25 S2_29 S2_30 S2_31 ').split(),
    'b': (
        'PR_3 S1_2 K3 BA_1 S1_0 S1_1 S1_3 BA_2 S2_2 S1_7 S1_5 S1_4 S1_6 S2_3 S2_0 S2_1 BA_3 S1_8 BA_4 BA_0 '
        'S1_9 PR_4 PR_1 K0 BB_0 S1_10 K2 S1_11 Q0 PR_0 S2_4 BB_1 K1 BC1_2 BC1_4 BC1_3 PR_2 S2_5 S2_6 S1_13 '
        'S1_12 S1_14 S2_7 S1_15 BC1_0 BC1_1 S2_10 S2_11 S2_8 S2_9 F0 S1_18 S1_17 S1_16 S1_19 BC2_1 S2_15 '
        'S2_13 Q2 BC2_2 S2_12 S2_14 S1_20 S1_22 S2_17 BC2_0 S1_21 BC2_3 F1 S1_23 S2_18 Q1 S2_19 S2_16 O0 '
        'S1_27 S1_25 S1_26 S2_22 S2_20 S1_24 BC3_1 BC3_2 BC2_4 S2_23 BC3_4 BC3_0 S1_28 S2_21 S1_31 S1_30 '
        'S1_29 BC3_3 O1 S2_24 S2_27 Q3 S2_25 S2_26 S2_31 S2_28 S2_30 S2_29 ').split(),
    'it15': (
        'S1_1 S1_13 S1_3 S1_0 S1_5 S1_6 S1_7 S1_2 S1_4 S2_0 O0 S2_1 S2_2 S1_8 S2_3 S1_10 S1_9 S1_11 S2_4 S2_6 '
        'S2_7 S1_12 S2_5 S2_8 S1_14 S1_15 S2_10 S2_11 S1_16 S2_9 S1_17 S1_18 S1_19 S2_12 S2_13 S2_15 S1_20 '
        'S1_22 S1_21 S1_23 S2_16 S2_14 S2_17 S2_19 S1_24 S1_25 S1_26 S1_27 S2_20 S2_22 S2_23 S1_28 S1_31 '
        'S1_29 S1_30 S2_21 S2_24 S2_25 S2_26 S2_27 O1 S2_18 S2_30 S2_28 S2_29 S2_31 ').split(),
}


def cmul(ar, ai, br, bi):
    return ar * br - ai * bi, ar * bi + ai * br


def csq(ar, ai):
    return ar * ar - ai * ai, (ar + ar) * ai


def bc16(x):
    return pltpu.bitcast(x, bf16)


def toi(x):
    return pltpu.bitcast(x, i32)


def pk(a, b):
    return pltpu.bitcast(pltpu.pack_elementwise([a, b], packed_dtype=bf16), i32)


def pk16(t):
    return jnp.concatenate([pk(t[r:r + 8], t[r + 8:r + 16]) for r in range(0, t.shape[0], 16)], 0)


def srl(x, n):
    return lax.shift_right_logical(x, jnp.int32(n))


def a8(x):
    return x if isinstance(x, int) else pl.multiple_of(x, 8)


def rowb(ref, base, r):
    return jnp.take_along_axis(ref[pl.ds(base, 8), :], jnp.full((8, 128), r, i32), axis=0)


def slot_of_chunk(m):
    p, m2 = m % 2, m // 2
    return 16 * p + 2 * (m2 % 8) + m2 // 8


def sincos(x):
    n = jnp.round(x * 0.6366197723675814)
    r = x - n * 1.5703125
    r = r - n * 4.837512969970703e-4
    r = r - n * 7.549790126404332e-8
    r = jnp.clip(r, -0.8, 0.8)
    q = n.astype(i32)
    z = r * r
    s = r + r * z * (-0.16666654611 + z * (0.0083321608736 + z * -0.00019515295891))
    c = 1.0 + z * (-0.5 + z * (0.04166664568298827 + z * (-0.001388731625493765 + z * 2.443315711809948e-5)))
    sw = (q & 1) != 0
    s2 = jnp.where(sw, c, s)
    c2 = jnp.where(sw, s, c)
    sn = jnp.where((q & 2) != 0, -s2, s2)
    cs = jnp.where(((q + 1) & 2) != 0, -c2, c2)
    return sn, cs


def ssm_prep(p, dt, dsc, put):
    lr = dt * p["Ar"]
    li = dt * p["Ai"]
    cr, ci = cmul(p["Cr"], p["Ci"], dt * p["Br"], dt * p["Bi"])
    eh = jnp.exp(lr * 0.5)
    sn, cs = sincos(li * 0.5)
    whr = eh * cs
    whi = eh * sn
    mx = jnp.maximum(jnp.abs(cr), jnp.abs(ci))
    eb = jnp.maximum(pltpu.bitcast(mx, i32), 0x01800000)
    eb = (eb - 0x00800000) & 0x7F000000
    inv = pltpu.bitcast(0x7E800000 - eb, f32)
    sm = pltpu.bitcast(srl(eb, 1) + 0x20000000, f32)
    a = cr * inv
    b = ci * inv
    x2 = jnp.maximum(a * a + b * b, 1e-30)
    y = lax.rsqrt(x2)
    x3 = (x2 * y + jnp.abs(a)) * 0.5
    y3 = lax.rsqrt(x3)
    t = x3 * y3
    q = b * (0.5 * y3)
    sr = jnp.where(a >= 0, t, jnp.abs(q)) * sm
    si = jnp.where(a >= 0, q, jnp.where(b < 0, -t, t)) * sm
    g0 = cmul(sr, si, whr, whi)
    k0 = jnp.sum(cr, axis=1, keepdims=True) + dsc
    dg = jnp.broadcast_to(k0, cr.shape)
    nxt = lax.broadcasted_iota(i32, (8, 128), 0) | 1
    dn = jnp.concatenate([jnp.take_along_axis(dg[r:r + 8], nxt, axis=0) for r in range(0, dg.shape[0], 8)], 0)
    dg = jnp.where(lax.broadcasted_iota(i32, dg.shape, 1) < 64, dg, dn)
    put('dg', pk(dg, dg))
    w1 = csq(whr, whi)
    put('w1', w1)
    w2 = csq(*w1)
    w4 = csq(*w2)
    w8 = csq(*w4)
    w16 = csq(*w8)
    put('w16', w16)
    put('w64', csq(*csq(*w16)))
    b0 = g0
    b1 = cmul(*b0, *w2)
    b2 = cmul(*b0, *w4)
    b3 = cmul(*b1, *w4)
    for k, b in enumerate((b0, b1, b2, b3)):
        put(k, b)
        put(4 + k, cmul(*b, *w8))


def kernel(x_hbm, w_hbm, wo_hbm, u_hbm, Ar_h, Ai_h, Br_h, Bi_h, Cr_h, Ci_h, ldt_h, dsk_h, o_hbm,
           zs, x_v, w_v, wo_v, u_v, par_v, ldt_v, dsk_v, oa_v, ob_v,
           wqvT, wk_i, woT, KS, VT_s, QT_s, OT_s,
           bbr, bbi, w1r, w1i, w16r, w16i, w64r, w64i, dgs, ut, yt, colt,
           sem_in, sem_oa, sem_ob, *scr):
    it_ = iter(scr)
    s_refs = [next(it_) for _ in range(NSS)]
    RTs, RLs, RSs, RZs, RYs, RTTs = [[next(it_) for _ in range(NGI)] for _ in range(6)]
    par_h = (Ar_h, Ai_h, Br_h, Bi_h, Cr_h, Ci_h)
    cp_w = [[pltpu.make_async_copy(w_hbm.at[:, 512 * j + 128 * g:512 * j + 128 * (g + 1)],
                                   w_v.at[:, 512 * j + 128 * g:512 * j + 128 * (g + 1)], sem_in.at[18 + 3 * g + j])
             for j in range(3)] for g in range(4)]
    XB = (0, 64, 128, 192, 384, 1024)
    x_h32 = x_hbm.bitcast(i32)
    u_h32 = u_hbm.bitcast(i32)
    o_h32 = o_hbm.bitcast(i32)
    cp_x = [pltpu.make_async_copy(x_h32.at[XB[k]:XB[k + 1]], x_v.at[XB[k]:XB[k + 1]], sem_in.at[k]) for k in range(5)]
    cp_small = [pltpu.make_async_copy(ldt_h, ldt_v, sem_in.at[5]),
                pltpu.make_async_copy(dsk_h, dsk_v, sem_in.at[6])]
    cp_par = [pltpu.make_async_copy(par_h[k].at[0:128], par_v.at[k, 0:128], sem_in.at[7 + k]) for k in range(6)]
    cp_par2 = [pltpu.make_async_copy(par_h[k].at[128:512], par_v.at[k, 128:512], sem_in.at[30 + k]) for k in range(6)]
    cp_wo = pltpu.make_async_copy(wo_hbm, wo_v, sem_in.at[13])

    def cp_u(cb):
        c0 = cb * 128 if isinstance(cb, int) else pl.multiple_of(cb * 128, 128)
        return pltpu.make_async_copy(u_h32.at[:, pl.ds(c0, 128)], u_v.at[:, pl.ds(c0, 128)], sem_in.at[14 + cb])
    for c in ([cp_x[0]] + cp_w[0] + cp_w[1] + [cp_x[1]] + cp_w[2] + cp_w[3] + cp_small + [cp_x[2]] + cp_par
              + [cp_wo, cp_u(0), cp_x[3]] + cp_par2 + [cp_u(1), cp_u(2), cp_u(3), cp_x[4]]):
        c.start()

    def zinit(i, c):
        zs[i] = 0
        return c
    lax.fori_loop(0, 2, zinit, 0)
    z0 = pl.multiple_of(zs[0], 128)
    z1 = pl.multiple_of(zs[1], 128)

    for k in range(6):
        par_v[k, 512:576, :] = jnp.zeros((64, 128), bf16)
    colt[512:576, :] = jnp.zeros((64, 256), f32)
    for m2 in range(16):
        ut[m2 * PITCH + 253:m2 * PITCH + 261, :] = jnp.zeros((8, 128), i32)
    lane = lax.broadcasted_iota(i32, (8, 128), 1)
    sub = lax.broadcasted_iota(i32, (8, 128), 0)
    rev = 7 - sub
    lg = srl(lane, 4)
    l16 = lane & 15
    mbit = [(lg & (1 << t)) != 0 for t in range(3)]
    mA = (2 * sub) <= l16
    mB = (2 * sub + 1) <= l16
    Mw = jnp.where(mA, jnp.int32(0xFFFF), 0) | jnp.where(mB, jnp.int32(-65536), 0)
    l64 = lane & 63
    mdiag = [jnp.where(l64 == 63 - 16 * a - 2 * sub, jnp.int32(0xFFFF), 0)
             | jnp.where(l64 == 62 - 16 * a - 2 * sub, jnp.int32(-65536), 0) for a in range(4)]
    mtri = [jnp.where(l64 > 63 - 16 * a - 2 * sub, jnp.int32(0xFFFF), 0)
            | jnp.where(l64 > 62 - 16 * a - 2 * sub, jnp.int32(-65536), 0) for a in range(4)]

    def mk_colt():
        dtrow = jnp.exp(ldt_v[...].reshape(1, 512).astype(f32)).astype(bf16).astype(f32)
        dsrow = dsk_v[...].reshape(1, 512).astype(f32)
        for k in range(4):
            colt[128 * k:128 * (k + 1), 0:128] = jnp.broadcast_to(dtrow[:, 128 * k:128 * (k + 1)], (128, 128)).T
            colt[128 * k:128 * (k + 1), 128:256] = jnp.broadcast_to(dsrow[:, 128 * k:128 * (k + 1)], (128, 128)).T

    def prep(gi, go, n=NGI):
        names = ("Ar", "Ai", "Br", "Bi", "Cr", "Ci")
        p = {}
        g0_ = gi + go
        nl = 16 * ((n + 2) // 2)
        if isinstance(gi, int):
            for kk, nm in enumerate(names):
                p[nm] = par_v[kk, pl.ds((g0_ // 2) * 16, nl), :].astype(f32)[(g0_ % 2) * 8:(g0_ % 2) * 8 + 8 * n]
        else:
            r16 = pl.multiple_of(srl(g0_, 1) * 16, 16)
            odd = (g0_ & 1) == 1
            for kk, nm in enumerate(names):
                v = par_v[kk, pl.ds(r16, nl), :].astype(f32)
                p[nm] = jnp.where(odd, v[8:8 + 8 * n], v[:8 * n])
        gw = a8(gi * 8 + go * 8)

        def put(key, v):
            if key == 'dg':
                dgs[pl.ds(gw, 8 * n), :] = v
            elif isinstance(key, str):
                rr, ri = {'w1': (w1r, w1i), 'w16': (w16r, w16i), 'w64': (w64r, w64i)}[key]
                rr[pl.ds(gw, 8 * n), :] = v[0]
                ri[pl.ds(gw, 8 * n), :] = v[1]
            else:
                for k in range(n):
                    bbr[pl.ds(gi * 72 + (go * 72 + 72 * k + key), 8, stride=9), :] = v[0][8 * k:8 * k + 8]
                    bbi[pl.ds(gi * 72 + (go * 72 + 72 * k + key), 8, stride=9), :] = v[1][8 * k:8 * k + 8]
        ssm_prep(p, colt[pl.ds(gw, 8 * n), 0:128], colt[pl.ds(gw, 8 * n), 128:129], put)

    def ut_tile(m2, cb):
        c0 = pl.multiple_of(cb * 128, 128)
        pcs = []
        for v2 in range(8):
            v = (v2 // 4) * 4 + (3 - v2 % 4)
            t = jnp.take_along_axis(u_v[m2 * 64 + 8 * v:m2 * 64 + 8 * v + 8, pl.ds(c0, 128)], rev, axis=0)
            pcs.append((t << 16) | srl(t, 16))
        x = bc16(jnp.concatenate(pcs, axis=0))
        ut[pl.ds(m2 * PITCH + 64 * cb, 64), :] = toi(x.T)

    def stageA(gi, go, k):
        RT, RL, RS = RTs[k], RLs[k], RSs[k]
        gb = a8(gi * 8 + (go + k) * 8)
        for r in range(8):
            o9 = gi * 72 + ((go + k) * 72 + 9 * r)
            e0 = (bbr[pl.ds(o9, 8), :], bbi[pl.ds(o9, 8), :])
            w1 = (rowb(w1r, gb, r), rowb(w1i, gb, r))
            w16 = (rowb(w16r, gb, r), rowb(w16i, gb, r))
            e1 = cmul(*e0, *w1)
            vr = []
            vi = []
            for a in range(4):
                vr.append(pk(e0[0], e1[0]))
                vi.append(pk(e0[1], e1[1]))
                if a < 3:
                    e0 = cmul(*e0, *w16)
                    e1 = cmul(*e1, *w16)
            Vr = jnp.concatenate(vr, 0)
            Vi = jnp.concatenate(vi, 0)
            RT[pl.ds(z0 + 64 * r, 32), :] = Vr
            RT[pl.ds(z0 + 64 * r + 32, 32), :] = Vi
            if r % 2 == 0:
                dp = gi * 4 + ((go + k) * 4 + r // 2)
                A_ = ut[pl.ds(dp, 8, stride=PITCH), :]
                B_ = ut[pl.ds(dp + 8 * PITCH, 8, stride=PITCH), :]
                X = Xe = (A_ & 0xFFFF) | (B_ << 16)
            else:
                X = srl(A_, 16) | (B_ & jnp.int32(-65536))
                RL[pl.ds(z0 + 8 * (r - 1), 16), :] = jnp.concatenate(
                    [jnp.where(mbit[2], pltpu.roll(X, 64, 1), Xe), jnp.where(mbit[2], X, pltpu.roll(Xe, 64, 1))], 0)
            L = jnp.concatenate([jnp.where(mbit[2], 0, X), jnp.where(mbit[2], X, 0)], 0)
            Lb = bc16(L)
            Sr = jnp.dot(Lb, bc16(jnp.concatenate([Vr, Vr], 0)), preferred_element_type=f32)
            Si = jnp.dot(Lb, bc16(jnp.concatenate([Vi, Vi], 0)), preferred_element_type=f32)
            RS[pl.ds(z0 + 66 * r, 32), :] = Sr
            RS[pl.ds(z0 + 66 * r + 33, 32), :] = Si

    def stageB(gi, go, ks):
        n = len(ks)
        gbs = [a8(gi * 8 + (go + k) * 8) for k in ks]
        w = [(w64r[pl.ds(gb, 8), :], w64i[pl.ds(gb, 8), :]) for gb in gbs]
        z = [None] * n
        for m in range(32):
            s = slot_of_chunk(m)
            for j, k in enumerate(ks):
                RS, RZ = RSs[k], RZs[k]
                if m == 0:
                    RZ[pl.ds(z0 + s, 8, stride=66), :] = bbr[pl.ds(gi * 72 + (go + k) * 72, 8, stride=9), :]
                    RZ[pl.ds(z0 + 33 + s, 8, stride=66), :] = bbi[pl.ds(gi * 72 + (go + k) * 72, 8, stride=9), :]
                else:
                    RZ[pl.ds(z0 + s, 8, stride=66), :] = z[j][0]
                    RZ[pl.ds(z0 + 33 + s, 8, stride=66), :] = z[j][1]
                if m < 31:
                    sr = RS[pl.ds(z1 + s, 8, stride=66), :]
                    si = RS[pl.ds(z1 + 33 + s, 8, stride=66), :]
                    if m == 0:
                        z[j] = (sr, si)
                    else:
                        tr, ti = cmul(*z[j], *w[j])
                        z[j] = (tr + sr, ti + si)

    def stageC1(gi, go, k):
        nt = (((1,), (1,)), ((), ()))
        RT, RZ, RY = RTs[k], RZs[k], RYs[k]
        for r in range(8):
            Vr = bc16(RT[pl.ds(z1 + 64 * r, 32), :])
            Vi = bc16(RT[pl.ds(z1 + 64 * r + 32, 32), :])
            Zr = RZ[pl.ds(z1 + 66 * r, 32), :].astype(bf16)
            Zi = RZ[pl.ds(z1 + 66 * r + 33, 32), :].astype(bf16)
            yi = (lax.dot_general(Zr, Vr, nt, preferred_element_type=f32)
                  - lax.dot_general(Zi, Vi, nt, preferred_element_type=f32))
            if r % 2 == 0:
                ye = yi
            else:
                RY[pl.ds(z0 + 16 * (r - 1), 32), :] = jnp.concatenate([ye, yi], axis=1)

    def stageC2(gi, go, k):
        RY, RTT = RYs[k], RTTs[k]
        gb = a8(gi * 8 + (go + k) * 8)
        for r in range(0, 8, 2):
            k1 = jnp.take_along_axis(RY[pl.ds(z1 + 16 * r, 8), :], jnp.zeros((8, 128), i32), axis=0)
            src = pk(pltpu.roll(k1, 1, 1), k1)
            dg = rowb(dgs, gb, r)
            Te = []
            To = []
            for a in range(4):
                t = pltpu.roll(src, 49 - 16 * a, 1, stride=2, stride_axis=0)
                t = jnp.take_along_axis(t, rev, axis=0)
                t = (t & mtri[a]) | (dg & mdiag[a])
                Te.append(jnp.where(mbit[2], 0, t))
                To.append(jnp.where(mbit[2], t, 0))
            RTT[pl.ds(z0 + 32 * r, 64), :] = jnp.concatenate(Te + To, 0)

    def stageC3(gi, go, k):
        RL, RY, RTT = RLs[k], RYs[k], RTTs[k]
        for r in range(0, 8, 2):
            Lb = bc16(RL[pl.ds(z1 + 8 * r, 16), :])
            y = jnp.dot(Lb, bc16(RTT[pl.ds(z1 + 32 * r, 64), :]), preferred_element_type=f32)
            yi = RY[pl.ds(z1 + 16 * r, 32), :]
            y = y + jnp.concatenate([jnp.where(sub == 0, 0.0, yi[0:8]), yi[8:32]], 0)
            dp = gi * 4 + ((go + k) * 4 + r // 2)
            for hf in range(2):
                y0 = y[8 * hf:8 * hf + 8]
                y1 = y[16 + 8 * hf:24 + 8 * hf]
                w = jnp.where(mbit[2], pk(pltpu.roll(y1, 64, 1), y1), pk(y0, pltpu.roll(y0, 64, 1)))
                yt[pl.ds(dp + 8 * hf * PITCH, 8, stride=PITCH), :] = w

    def fin_tile(rho, db):
        if isinstance(rho, int):
            r0 = (rho // 2 + 8 * (rho % 2)) * 64
        else:
            r0 = pl.multiple_of((srl(rho, 1) + 8 * (rho & 1)) * 64, 64)
        x = bc16(yt[pl.ds(rho * PITCH + 64 * db, 64), :])
        c0 = pl.multiple_of(db * 128, 128)
        ob_v[pl.ds(r0, 64), pl.ds(c0, 128)] = toi(x.T)

    def cp_ob(db):
        c0 = pl.multiple_of(db * 128, 128)
        return pltpu.make_async_copy(ob_v.at[:, pl.ds(c0, 128)], o_h32.at[:, pl.ds(512 + c0, 128)], sem_ob.at[db])

    def Bjobs(i):
        P_ = functools.partial
        gi = i * NGI
        go = -6
        ng = NGI
        if isinstance(i, int) and i == 1:
            gi, go, ng = 0, 0, 4
        jobs = []
        for n, f in (("BA", stageA), ("BC1", stageC1), ("BC2", stageC2), ("BC3", stageC3)):
            jobs += [('%s_%d' % (n, k), P_(f, gi, go, k)) for k in range(ng)]
        jobs += [('BB_0', P_(stageB, gi, go, (0, 1, 2))), ('BB_1', P_(stageB, gi, go, tuple(range(3, ng))))]
        return jobs

    nt = (((1,), (1,)), ((), ()))

    wperm = [(2 * (sub & 3), 2 * (sub & 3) + 1, sub < 4),
             (4 * (sub & 1) + srl(sub, 2), 4 * (sub & 1) + srl(sub, 2) + 2, (sub & 2) == 0)]

    def wprep(g):
        gs = slice(128 * g, 128 * (g + 1))
        wk_i[:, gs] = toi(w_v[:, 512 + 128 * g:512 + 128 * (g + 1)])
        for j in range(2):
            for ct in range(4):
                n_ = toi(w_v[ct * 128:(ct + 1) * 128, 1024 * j + 128 * g:1024 * j + 128 * (g + 1)].T)
                pa, pb, ml = wperm[j]
                out = []
                for v in range(8):
                    a_ = jnp.take_along_axis(n_[8 * v:8 * v + 8], pa, axis=0)
                    b_ = jnp.take_along_axis(n_[8 * v:8 * v + 8], pb, axis=0)
                    out.append(jnp.where(ml, (a_ & 0xFFFF) | (b_ << 16), srl(a_, 16) | (b_ & jnp.int32(-65536))))
                wqvT[256 * j + 64 * g:256 * j + 64 * (g + 1), ct * 128:(ct + 1) * 128] = jnp.concatenate(out, 0)

    def woprep():
        for ct in range(4):
            for ht in range(4):
                woT[ht * 64:(ht + 1) * 64, ct * 128:(ct + 1) * 128] = toi(
                    wo_v[ct * 128:(ct + 1) * 128, ht * 128:(ht + 1) * 128].T)

    def projK(i, off, g0, ng=1):
        xi = x_v[pl.ds(pl.multiple_of(i * 64 + off * 64, 64), 64), :]
        lo = pltpu.bitcast(xi << 16, f32)
        hi = pltpu.bitcast(xi & jnp.int32(-65536), f32)
        xp = jnp.concatenate([v[8 * j:8 * j + 8] for j in range(8) for v in (lo, hi)], 0).astype(bf16)
        k = jnp.dot(xp, bc16(wk_i[:, 128 * g0:128 * (g0 + ng)]), preferred_element_type=f32)
        kis = toi(k.astype(bf16))
        for gg in range(ng):
            g = g0 + gg
            cur = [kis[8 * b:8 * b + 8, 128 * gg:128 * (gg + 1)] for b in range(8)]
            for t in range(3):
                d = 1 << t
                new = list(cur)
                for b0 in range(8):
                    if b0 & d:
                        continue
                    b1 = b0 + d
                    new[b0] = jnp.where(mbit[t], pltpu.roll(cur[b1], 16 * d, 1), cur[b0])
                    new[b1] = jnp.where(mbit[t], cur[b1], pltpu.roll(cur[b0], 128 - 16 * d, 1))
                cur = new
            ih = i * 64
            hbs = [(8 * g + hh) * NA * 8 + 64 + 64 * off for hh in range(8)]
            first = isinstance(i, int) and i + off == 0
            for hh in range(8):
                KS[pl.ds(ih + hbs[hh] + 64, 8), :] = cur[hh]
                if first:
                    KS[pl.ds(ih + hbs[hh], 8), :] = cur[hh]
            for j in range(1, 8):
                mj = lg < 8 - j
                for hh in range(8):
                    rot = pltpu.roll(cur[hh], 128 - 16 * j, 1)
                    KS[pl.ds(ih + hbs[hh] + 64 + 8 * j, 8), :] = rot
                    KS[pl.ds(ih + hbs[hh] + 8 * j, 8), :] = (
                        rot if first else jnp.where(mj, KS[pl.ds(ih + hbs[hh] + 8 * j, 8), :], rot))

    def projQV(i, off, r0, nr):
        xb = bc16(x_v[pl.ds(pl.multiple_of(i * 64 + off * 64, 64), 64), :])
        w = bc16(wqvT[r0:r0 + nr, :])
        t = lax.dot_general(w, xb, nt, preferred_element_type=f32)
        if r0 < 256:
            t = t * SCALE
            QT_s[pl.ds(i * 256 + (off * 256 + r0), nr), :] = pk16(t)
        else:
            VT_s[pl.ds(i * 256 + (off * 256 + r0 - 256), nr), :] = pk16(t)

    def cp_oa(i):
        rows = pl.ds(pl.multiple_of(i * 64, 64), 64)
        return pltpu.make_async_copy(oa_v.at[rows, :], o_h32.at[rows, 0:512], sem_oa.at[i])

    def outp(i, off, hf):
        ot = bc16(OT_s[pl.ds(i * 256 + off * 256, 256), :])
        o = jnp.dot(bc16(woT[128 * hf:128 * (hf + 1), :]), ot, preferred_element_type=f32).astype(bf16).T
        oa_v[pl.ds(pl.multiple_of(i * 64 + off * 64, 64), 64), 256 * hf:256 * (hf + 1)] = toi(o)

    def attn(i, kind, jobs, seq):
        amin = {0: 9, 1: 1, 2: 0}[kind]
        ms = {}
        order = ([0, 16] if kind == 2 else [16]) + list(range(max(amin, 1), 16))
        nrow = 16 * (len(order) - (1 if kind == 2 else 0))
        i64 = i * 64
        i256 = i * 256

        def stage1(h):
            s_s = s_refs[h % NSS]
            qh = QT_s[pl.ds(i256 + h * 8, 8), :]
            W = bc16(jnp.concatenate([jnp.where(lg == s, qh, 0) for s in range(8)], 0))
            lhs = jnp.concatenate([KS[pl.ds(i64 + (h * NA * 8 + 8 * a), 8), :] for a in order], 0)
            st = jnp.dot(bc16(lhs), W, preferred_element_type=f32)
            if kind == 2:
                tA = jnp.where(mA, st[16:24], st[0:8])
                tB = jnp.where(mB, st[24:32], st[8:16])
                off = 32
            else:
                tA = jnp.where(mA, st[0:8], NEG)
                tB = jnp.where(mB, st[8:16], NEG)
                off = 16
            s_s[pl.ds(z0, 16), :] = jnp.concatenate([tA, tB], 0)
            m = jnp.maximum(tA, tB)
            for n, a in enumerate(order[(2 if kind == 2 else 1):]):
                t = st[off + 16 * n:off + 16 * n + 16]
                thr = 16 - 8 * kind - a
                if kind < 2 and thr > 0:
                    t = jnp.where(jnp.concatenate([lg, lg], 0) >= thr, t, NEG)
                s_s[pl.ds(z0 + 16 + 16 * n, 16), :] = t
                m = jnp.maximum(m, jnp.maximum(t[0:8], t[8:16]))
            ms[h] = jnp.max(m, axis=0, keepdims=True)

        def stage2(h):
            s_s = s_refs[h % NSS]
            m = ms[h]
            rest = order[2:] if kind == 2 else order[1:]
            slot = {a: 1 + n for n, a in enumerate(rest)}
            slot[16] = 0
            acc = {}
            memo = {}

            def word(n):
                if ('w', n) not in memo:
                    p = jnp.exp2(s_s[pl.ds(z1 + 16 * n, 16), :] - m)
                    t = p[0:8] + p[8:16]
                    k = memo['cnt'] = memo.get('cnt', -1) + 1
                    acc[k % NACC] = t if (k % NACC) not in acc else acc[k % NACC] + t
                    memo[('w', n)] = pk(p[0:8], p[8:16])
                return memo[('w', n)]

            def x0(a):
                if a == 16:
                    return word(0) & Mw if kind == 2 else word(0)
                if a == 0 and kind == 2:
                    return word(0) & ~Mw
                return word(slot[a]) if a in slot else None

            def get(t, a):
                if (t, a) in memo:
                    return memo[(t, a)]
                if t == 0:
                    r = x0(a) if 0 <= a <= 16 else None
                    if 0 <= a - LOOK <= 16 and r is not None:
                        x0(a - LOOK)
                else:
                    d = 1 << (t - 1)
                    lo_ = get(t - 1, a)
                    hi_ = get(t - 1, a - d)
                    if hi_ is None and lo_ is None:
                        r = None
                    else:
                        r = jnp.where(mbit[t - 1], 0 if hi_ is None else hi_, 0 if lo_ is None else lo_)
                memo[(t, a)] = r
                return r

            ot = None
            for tt in range(2, 1 - kind, -1):
                rows = [get(3, a) for a in range(8 * tt + 7, 8 * tt - 1, -1)][::-1]
                Pm = bc16(jnp.concatenate([jnp.zeros((8, 128), i32) if x is None else x for x in rows], 0))
                vt = bc16(VT_s[pl.ds(i256 + ((tt - 2) * 256 + h * 8), 8), :])
                o_ = jnp.dot(vt, Pm, preferred_element_type=f32)
                ot = o_ if ot is None else ot + o_
            l = functools.reduce(lambda a_, b_: a_ + b_, acc.values())
            l = jnp.sum(l, axis=0, keepdims=True)
            rc = pl.reciprocal(l, approx=True)
            rc = rc * (2.0 - l * rc)
            ot = ot * rc
            OT_s[pl.ds(i256 + h * 8, 8), :] = pk16(ot)

        jd = dict(jobs)
        for it in seq:
            if it.startswith('S1_'):
                stage1(int(it[3:]))
            elif it.startswith('S2_'):
                stage2(int(it[3:]))
            elif it in jd:
                jd.pop(it)()
        assert all(k.startswith('PR') for k in jd), list(jd)

    P_ = functools.partial

    def Pj(i, off):
        return ([('K%d' % g, P_(projK, i, off, g)) for g in range(4)]
                + [('Q%d' % c, P_(projQV, i, off, 128 * c, 128)) for c in range(4)])

    def Oj(i, off):
        return [('O%d' % hf, P_(outp, i, off, hf)) for hf in range(2)]

    def ut_jobs(cb, m2s, tag):
        def run(ms_):
            for m2 in ms_:
                ut_tile(m2, cb)
        return [('%s%d' % (tag, n), P_(run, m2s[4 * n:4 * n + 4])) for n in range((len(m2s) + 3) // 4)]

    def w_0(g):
        if g == 0:
            cp_x[0].wait()
        for c in cp_w[g]:
            c.wait()

    def w_a():
        for c in cp_small + [cp_x[2], cp_wo] + cp_par + [cp_u(0)]:
            c.wait()

    def late_prep(i):
        return ([('PREP', P_(prep, i * NGI, -1))] + [('PR_%d' % k, P_(prep, i * NGI, k - 1, 1)) for k in range(NGI)])

    j0 = [('WQ%d' % g, P_(w_0, g)) for g in range(4)] + [('WX', cp_x[1].wait)]
    j0 += [('PW%d' % g, P_(wprep, g)) for g in range(4)]
    for o, tag in ((0, 'A'), (1, '')):
        j0 += [('K%s%d' % (tag, g), P_(projK, 0, o, g)) for g in range(4)]
        j0 += [('Q%s%d' % (tag, g), P_(projQV, 0, o, 64 * g, 64)) for g in range(4)]
        j0 += [('V%s%d' % (tag, g), P_(projQV, 0, o, 256 + 64 * g, 64)) for g in range(4)]
    attn(0, 0, j0, SEQS['it0'])
    attn(1, 1, ut_jobs(0, list(range(16)), 'U') + [('WA', w_a), ('WOP', woprep), ('COLT', mk_colt), ('PRE', lambda: prep(0, 0, 4)),
                                                  ('W1', lambda: [c.wait() for c in [cp_x[3]] + cp_par2])]
         + Pj(1, 1) + Oj(1, -1) + Bjobs(1) + late_prep(1), SEQS['it1'])
    cp_oa(0).start()

    def body_a(i, c):
        attn(i, 2, Pj(i, 1) + Oj(i, -1) + Bjobs(i) + late_prep(i) + ut_jobs(i - 1, list(range(16)), 'U')
             + [('WU', lambda: cp_u(i - 1).wait())], SEQS['a'])
        cp_oa(i - 1).start()
        return c

    lax.fori_loop(2, 5, body_a, 0)
    cp_x[4].wait()

    def body_b(i, c):
        db = lax.div(i - 5, 3)
        j = (i - 5) - 3 * db

        def fj(ks):
            for k in ks:
                fin_tile(jnp.minimum(6 * j + k, 15), db)
        attn(i, 2, Pj(i, 1) + Oj(i, -1) + Bjobs(i) + late_prep(i) + [('F0', P_(fj, (0, 1, 2))), ('F1', P_(fj, (3, 4, 5)))],
             SEQS['b'])
        cp_oa(i - 1).start()

        @pl.when(j == 2)
        def _():
            cp_ob(db).start()
        return c

    lax.fori_loop(5, 14, body_b, 0)

    def fin3(rs):
        for rho in rs:
            fin_tile(rho, 3)
    attn(14, 2, Pj(14, 1) + Oj(14, -1) + [('F%d' % n, P_(fin3, range(4 * n, 4 * n + 4))) for n in range(4)],
         SEQS['it14'])
    cp_oa(13).start()
    cp_ob(3).start()
    attn(15, 2, Oj(15, -1), SEQS['it15'])
    outp(15, 0, 0)
    outp(15, 0, 1)
    cp_oa(14).start()
    cp_oa(15).start()
    for db in range(4):
        cp_ob(db).wait()

    def wbody(i, c):
        cp_oa(i).wait()
        return c
    lax.fori_loop(0, 16, wbody, 0)


@jax.jit
def pallas_concat_heads__sliding_block__ssm_conv_s4__prompt_kernel(
    A_x, A_wqkv, A_wo, B_u, B_A_re, B_A_im, B_B_re, B_B_im, B_C_re, B_C_im, B_log_dt, B_Dskip,
):
    V = pltpu.VMEM
    NR = 8 * 14 * NGI
    scr = [
        pltpu.SMEM((2,), i32),
        V((S_LEN // 2, 512), i32), V((512, 1536), bf16), V((512, 512), bf16), V((S_LEN // 2, 512), i32),
        V((6, 576, 128), bf16), V((512,), bf16), V((512,), bf16), V((S_LEN // 2, 512), i32), V((S_LEN // 2, 512), i32),
        V((512, 512), i32), V((256, 512), i32), V((256, 512), i32), V((32 * NA * 8, 128), i32),
        V((16 * 256, 128), i32), V((16 * 256, 128), i32), V((16 * 256, 128), i32),
        V((NR * 9, 128), f32), V((NR * 9, 128), f32)] + [V((NR, 128), f32)] * 6 + [
        V((NR, 128), i32), V((16 * PITCH, 128), i32), V((16 * PITCH, 128), i32), V((576, 256), f32),
        pltpu.SemaphoreType.DMA((36,)), pltpu.SemaphoreType.DMA((16,)), pltpu.SemaphoreType.DMA((4,)),
    ]
    scr += [V((256, 128), f32)] * NSS
    for sh in [V((8 * 64, 128), i32), V((8 * 16, 128), i32), V((8 * 66, 128), f32), V((8 * 66, 128), f32),
               V((8 * 32, 128), f32), V((8 * 32, 128), i32)]:
        scr += [sh] * NGI
    out = pl.pallas_call(
        kernel,
        out_shape=jax.ShapeDtypeStruct((S_LEN, 1024), bf16),
        in_specs=[pl.BlockSpec(memory_space=pl.ANY)] * 12,
        out_specs=pl.BlockSpec(memory_space=pl.ANY),
        scratch_shapes=scr,
        compiler_params=pltpu.CompilerParams(vmem_limit_bytes=100 * 1024 * 1024),
        name="fused",
    )(A_x.reshape(S_LEN, 512), A_wqkv, A_wo, B_u.reshape(S_LEN, 512), B_A_re, B_A_im, B_B_re, B_B_im,
      B_C_re, B_C_im, B_log_dt, B_Dskip)
    return out.reshape(1, S_LEN, 1024)
```
